```python
import jax
import jax.numpy as jnp

def _softmax(x, axis=-1):
    return jax.nn.softmax(x, axis=axis)
def _gelu(x):
    return jax.nn.gelu(x, approximate=True)
def _silu(x):
    return jax.nn.silu(x)
def _sigmoid(x):
    return jax.nn.sigmoid(x)
def _layernorm(x, axis=-1, eps=1e-5):
    m = jnp.mean(x, axis=axis, keepdims=True)
    v = jnp.var(x, axis=axis, keepdims=True)
    return (x - m) / jnp.sqrt(v + eps)
def _scatter_add(tgt, idx, src, axis=0):
    return tgt.at[idx].add(src)
def _segment_sum(src, seg, n):
    return jax.ops.segment_sum(src, seg, n)
class _Rng:
    def __init__(self, key):
        self._k = key
    def _next(self):
        self._k, sub = jax.random.split(self._k)
        return sub
    def normal(self, shape):
        return jax.random.normal(self._next(), shape, dtype=jnp.bfloat16)
    def randint(self, lo, hi, shape):
        return jax.random.randint(self._next(), shape, lo, hi, dtype=jnp.int32)
    def uniform(self, shape, lo=0.0, hi=1.0):
        return jax.random.uniform(self._next(), shape, jnp.bfloat16, lo, hi)
    def permutation(self, n):
        return jax.random.permutation(self._next(), n)


kernel_name = 'sequential_preLN__sliding_local_dilated__moe_arch_mod__prompt'

def setup_inputs():
    _rng = _Rng(jax.random.key(int.from_bytes(__import__("os").urandom(4), "little")))
    _w = (lambda a: (lambda t: t.astype(jnp.bfloat16) if jnp.issubdtype(t.dtype, jnp.floating) else t)(jnp.asarray(a)))
    def _A_setup():
        B, S, D = 1, 2048, 640
        return {
            "x": _w((lambda *s: _rng.normal(s) * 0.05)(B, S, D)),
            "wqkv": _w((lambda *s: _rng.normal(s) * 0.05)(D, 3 * D)),
            "wo": _w((lambda *s: _rng.normal(s) * 0.05)(D, D)),
        }
    _A_in = _A_setup()

    def _B_setup():
        B, S, D, F, C = 1, 2048, 640, 1536, 1
        return {
            "x": _w((lambda *s: _rng.normal(s) * 0.05)(B, S, D)),
            "w_r": _w((lambda *s: _rng.normal(s) * 0.05)(D)),
            "w_gate": _w((lambda *s: _rng.normal(s) * 0.05)(D, F)),
            "w_up": _w((lambda *s: _rng.normal(s) * 0.05)(D, F)),
            "w_down": _w((lambda *s: _rng.normal(s) * 0.05)(F, D)),
        }
    _B_in = _B_setup()

    return {
        "A_x": _A_in["x"],
        "A_wqkv": _A_in["wqkv"],
        "A_wo": _A_in["wo"],
        "B_x": _B_in["x"],
        "B_w_r": _B_in["w_r"],
        "B_w_gate": _B_in["w_gate"],
        "B_w_up": _B_in["w_up"],
        "B_w_down": _B_in["w_down"],
    }

def reference(A_x, A_wqkv, A_wo, B_x, B_w_r, B_w_gate, B_w_up, B_w_down):
    def _A_ref(x, wqkv, wo):
        B, S, D = x.shape
        H = 32; Dh = D // H
        W, dil = 8, 2
        qkv = (lambda x, *d: x.transpose(*d))((x @ wqkv).reshape(B, S, 3, H, Dh), 2, 0, 3, 1, 4)
        q, k, v = qkv[0], qkv[1], qkv[2]
        scale = Dh ** -0.5
        pos = jnp.arange(S)
        off = jnp.arange(W) * dil
        idx = pos[:, None] - off[None, :]
        mask = idx >= 0
        idx_c = jnp.where(mask, idx, 0).reshape(-1)
        kg = k[:, :, idx_c, :].reshape(B, H, S, W, Dh)
        vg = v[:, :, idx_c, :].reshape(B, H, S, W, Dh)
        logits = jnp.einsum("bhsd,bhswd->bhsw", q, kg) * scale
        logits = jnp.where(mask[None, None, :, :], logits, -1e9)
        attn = _softmax(logits, axis=-1)
        o = jnp.einsum("bhsw,bhswd->bhsd", attn, vg)
        return (lambda x, *d: x.transpose(*d))(o, 0, 2, 1, 3).reshape(B, S, D) @ wo

    def _B_ref(x, w_r, w_gate, w_up, w_down):
        B, S, D = x.shape
        C = 1
        r = x @ w_r
        idx = jnp.argsort(-r, axis=-1)[:, :C]
        idx_e = jnp.repeat(idx.reshape(B, C, 1), D, axis=2)
        x_sel = jnp.take_along_axis(x, idx_e, axis=1)
        g = _silu(x_sel @ w_gate)
        u = x_sel @ w_up
        y = (g * u) @ w_down
        r_sel = _sigmoid(jnp.take_along_axis(r, idx, axis=1))
        y = y * r_sel.reshape(B, C, 1)
        b_off = (jnp.arange(B) * S).reshape(B, 1)
        flat_idx = (idx + b_off).reshape(B * C)
        zero = (x * 0.0).reshape(B * S, D)
        upd = _scatter_add(zero, flat_idx, y.reshape(B * C, D), axis=0)
        return x + upd.reshape(B, S, D)

    x = A_x
    h = x + _A_ref(_layernorm(x, axis=-1), A_wqkv, A_wo)
    h2 = h + _B_ref(_layernorm(h, axis=-1), B_w_r, B_w_gate, B_w_up, B_w_down)
    return h2
```

```python
import functools
import numpy as np
import jax
import jax.numpy as jnp
from jax import lax
import jax.experimental.pallas as pl
import jax.experimental.pallas.tpu as pltpu

S, D, H, DH, F = 2048, 640, 32, 20, 1536
NW, DIL = 8, 2
LT = D // 128
HALO = 16
f32, bf16, i32 = jnp.float32, jnp.bfloat16, jnp.int32
LOG2E = 1.4426950408889634


def make_kernel(T=256, ffn=True, flags=None, RA=16, outgrp="57", xwait=0, nofwd=0):
    NB = S // T

    def kern(z_ref, x_hbm, wqkv_hbm, wo_hbm, wr_ref, wg_hbm, wu_hbm, wd_hbm, out_hbm,
             x_v, wq_v, wo_v, wg_v, wu_v, wd_v, out_v,
             wp, wop, wof, xn, os_, xf, qs, ks, vs, hs, sems):
        P = functools.partial
        z = z_ref[0]
        def dz(off, n, bit, al=1):
            if nofwd & bit:
                return pl.ds(pl.multiple_of(off + al * z, al), n)
            return pl.ds(off, n)

        def x_copy(i):
            return pltpu.make_async_copy(x_hbm.at[pl.ds(i * T, T), :], x_v.at[pl.ds(i * T, T), :], sems.at[i])
        def out_copy(lo, hi):
            return pltpu.make_async_copy(out_v.at[pl.ds(lo * T, (hi - lo) * T), :], out_hbm.at[pl.ds(lo * T, (hi - lo) * T), :], sems.at[NB + lo])
        w_copies = [pltpu.make_async_copy(wqkv_hbm.at[:, pl.ds(s * D, D)], wq_v.at[s], sems.at[2 * NB + s]) for s in range(3)]
        wo_copy = pltpu.make_async_copy(wo_hbm, wo_v, sems.at[2 * NB + 3])
        wg_copy = pltpu.make_async_copy(wg_hbm, wg_v, sems.at[2 * NB + 4])
        wu_copy = pltpu.make_async_copy(wu_hbm, wu_v, sems.at[2 * NB + 5])
        wd_copy = pltpu.make_async_copy(wd_hbm, wd_v, sems.at[2 * NB + 6])
        x_copy(0).start()
        w_copies[0].start()
        w_copies[1].start()
        x_copy(1).start()
        w_copies[2].start()
        for i in range(2, NB):
            x_copy(i).start()
        wo_copy.start()
        if ffn:
            wg_copy.start(); wu_copy.start(); wd_copy.start()

        lane = lax.broadcasted_iota(i32, (8, 128), 1)

        def permute_w(sec):
            hh = lane & 31
            gg = lane >> 5
            for t in range(LT):
                c = hh * DH + 4 * t + gg
                src_lane = c & 127
                hp = (13 * ((lane >> 2) - t)) & 31
                cp = hp * DH + 4 * t + (lane & 3)
                tile_l = cp >> 7
                for r in range(D // 16):
                    srcs = [pltpu.bitcast(wq_v[sec, pl.ds(16 * r, 16), pl.ds(128 * u, 128)], i32) for u in range(LT)]
                    comb = srcs[0]
                    for u in range(1, LT):
                        comb = jnp.where(tile_l == u, srcs[u], comb)
                    wp[pl.ds(8 * r, 8), pl.ds(128 * (sec * LT + t), 128)] = jnp.take_along_axis(comb, src_lane, axis=1)

        def permute_wo():
            for u in range(LT):
                wof[u] = wo_v[:, pl.ds(128 * u, 128)].astype(f32)
            for u in range(LT):
                for d in range(DH):
                    blk_ = wof[u, pl.ds(d, H, stride=DH), :]
                    wop[pl.ds(16 * d, 16), pl.ds(128 * u, 128)] = pltpu.bitcast(blk_.astype(bf16), i32)

        def red(f, xs):
            xs = list(xs)
            while len(xs) > 1:
                nx = [f(xs[k], xs[k + 1]) for k in range(0, len(xs) - 1, 2)]
                if len(xs) % 2:
                    nx.append(xs[-1])
                xs = nx
            return xs[0]

        def ln(xs):
            m = jnp.sum(red(jnp.add, xs), axis=1, keepdims=True) * (1.0 / D)
            cs = [a - m for a in xs]
            var = jnp.sum(red(jnp.add, [a * a for a in cs]), axis=1, keepdims=True) * (1.0 / D)
            rs = lax.rsqrt(var + 1e-5)
            return [a * rs for a in cs]

        def s1_chunk(r0):
            xs = [x_v[pl.ds(r0, 16), pl.ds(128 * t, 128)].astype(f32) for t in range(LT)]
            ys = ln(xs)
            for t in range(LT):
                xn[pl.ds(r0 // 2, 8), pl.ds(128 * t, 128)] = pltpu.bitcast(ys[t].astype(bf16), i32)
                xf[t, pl.ds(r0, 16), :] = xs[t]

        def lhs(buf, i):
            return pltpu.bitcast(buf[dz(i * T // 2, T // 2, 1, 8), :], bf16)

        def s2_unit(i, n):
            sec, t = divmod(n, LT)
            res = jnp.dot(lhs(xn, i), pltpu.bitcast(wp[:, pl.ds(128 * n, 128)], bf16), preferred_element_type=f32)
            if sec == 0:
                qs[t, pl.ds(i * T, T), :] = res * (DH ** -0.5 * LOG2E)
            elif sec == 1:
                ks[t, pl.ds(HALO + i * T, T), :] = res
            else:
                vs[t, pl.ds(HALO + i * T, T), :] = res

        def s3_rows(r0, R):
            masked = r0 < HALO
            q = [qs[t, dz(r0, R, 8), :] for t in range(LT)]
            Ls = []
            for w in range(NW):
                p = red(jnp.add, [q[t] * ks[t, dz(HALO + r0 - DIL * w, R, 8), :] for t in range(LT)])
                p = p + pltpu.roll(p, 64, 1)
                p = p + pltpu.roll(p, 32, 1)
                if masked and w > 0:
                    row = lax.broadcasted_iota(i32, (R, 128), 0) + r0
                    p = jnp.where(row >= DIL * w, p, -1e9)
                Ls.append(p)
            m = red(jnp.maximum, Ls)
            es = [jnp.exp2(l - m) for l in Ls]
            inv = 1.0 / red(jnp.add, es)
            for t in range(LT):
                a = red(jnp.add, [es[w] * vs[t, dz(HALO + r0 - DIL * w, R, 16), :] for w in range(NW)]) * inv
                os_[pl.ds(r0 // 2, R // 2), pl.ds(128 * t, 128)] = pltpu.bitcast(a.astype(bf16), i32)

        wr = [wr_ref[:, pl.ds(128 * t, 128)] for t in range(LT)]
        best = [None, None]

        def s4_unit(i, n):
            res = jnp.dot(lhs(os_, i), pltpu.bitcast(wop[:, pl.ds(128 * n, 128)], bf16), preferred_element_type=f32)
            hs[n, pl.ds(i * T, T), :] = res + xf[n, dz(i * T, T, 4), :]

        def s4_chunk(r0):
            h = [hs[t, dz(r0, 16, 32), :] for t in range(LT)]
            ys = ln(h)
            rr = red(jnp.add, [ys[t] * wr[t] for t in range(LT)])
            rv = jnp.broadcast_to(jnp.sum(rr, axis=1, keepdims=True), (16, 128))
            idx = lax.broadcasted_iota(i32, (16, 128), 0) + r0
            if best[0] is None:
                best[0], best[1] = rv, idx
            else:
                gt = rv > best[0]
                best[0] = jnp.where(gt, rv, best[0])
                best[1] = jnp.where(gt, idx, best[1])
            for t in range(LT):
                out_v[pl.ds(r0, 16), pl.ds(128 * t, 128)] = (h[t] + ys[t]).astype(bf16)

        def merge(pools):
            tot = sum(len(p) for p in pools)
            idx = [0] * len(pools)
            mix = []
            for s in range(tot):
                bp, bv = None, None
                for pi, p in enumerate(pools):
                    if idx[pi] < len(p):
                        v = (idx[pi] + 0.5) / len(p)
                        if bv is None or v < bv:
                            bp, bv = pi, v
                mix.append(pools[bp][idx[bp]])
                idx[bp] += 1
            return mix

        def interleave(units, chunks):
            nu, nc = len(units), len(chunks)
            done = 0
            for u, fu in enumerate(units):
                fu()
                tgt = (u + 1) * nc // nu
                while done < tgt:
                    chunks[done]()
                    done += 1
            while done < nc:
                chunks[done]()
                done += 1

        for t in range(LT):
            ks[t, pl.ds(0, HALO), :] = jnp.zeros((HALO, 128), f32)
            vs[t, pl.ds(0, HALO), :] = jnp.zeros((HALO, 128), f32)

        x_copy(0).wait()
        for r in range(T // 16):
            s1_chunk(16 * r)
        started = []
        out_lo = 0
        for j in range(-1, NB + 1):
            units, chunks = [], []
            if j == xwait:
                for i in range(2, NB):
                    x_copy(i).wait()
                wo_copy.wait()
            if str(j) in outgrp:
                out_copy(out_lo, j - 1).start()
                started.append((out_lo, j - 1))
                out_lo = j - 1
            if 0 <= j - 1 < NB:
                units += [P(s4_unit, j - 1, n) for n in range(LT)]
            if 0 <= j + 1 < NB:
                if j == -1:
                    for sec in range(3):
                        units.append(w_copies[sec].wait)
                        if sec == 1:
                            units.append(x_copy(1).wait)
                        units.append(P(permute_w, sec))
                        units += [P(s2_unit, 0, sec * LT + t) for t in range(LT)]
                else:
                    units += [P(s2_unit, j + 1, n) for n in range(3 * LT)]
            att = [P(s3_rows, j * T + RA * r, RA) for r in range(T // RA)] if 0 <= j < NB else []
            ln1 = [P(s1_chunk, (j + 2) * T + 16 * r) for r in range(T // 16)] if 0 <= j + 2 < NB else []
            ln2 = [P(s4_chunk, (j - 1) * T + 16 * r) for r in range(T // 16)] if 0 <= j - 1 < NB else []
            extra = [permute_wo] if j == 0 else []
            na = len(att)
            pre = merge([att, ln1, extra])
            nwo = LT if 0 <= j - 1 < NB else 0
            ntot = len(pre) + len(ln2)
            k0 = min(len(pre), -(-nwo * ntot // max(1, len(units)))) if units else 0
            rest = merge([pre[k0:], ln2])
            if j == -1:
                for fu in units:
                    fu()
                for c in pre[:k0] + rest:
                    c()
            else:
                if units[:nwo]:
                    interleave(units[:nwo], pre[:k0])
                else:
                    for c in pre[:k0]:
                        c()
                if units[nwo:]:
                    interleave(units[nwo:], rest)
                else:
                    for c in rest:
                        c()

        if ffn:
            mx = jnp.max(best[0])
            sel = jnp.min(jnp.where(best[0] == mx, best[1], S))
            base = pl.multiple_of((sel >> 4) << 4, 16)
            h = [hs[t, pl.ds(base, 16), :] for t in range(LT)]
            ys = ln(h)
            row = lax.broadcasted_iota(i32, (16, 128), 0) + base
            is_sel = row == sel
            xs = jnp.concatenate([jnp.where(is_sel, y, 0.0) for y in ys], axis=1)
            xs = jnp.broadcast_to(jnp.sum(xs, axis=0, keepdims=True), (16, D)).astype(bf16)
            wg_copy.wait(); wu_copy.wait(); wd_copy.wait()
            out_copy(out_lo, NB).start()
            started.append((out_lo, NB))
            g = jnp.dot(xs, wg_v[...], preferred_element_type=f32)
            u = jnp.dot(xs, wu_v[...], preferred_element_type=f32)
            a = (g * jax.nn.sigmoid(g) * u).astype(bf16)
            y = jnp.dot(a, wd_v[...], preferred_element_type=f32)
            gt_ = jax.nn.sigmoid(jnp.full((16, 128), mx, f32))
            for (lo, hi) in started:
                out_copy(lo, hi).wait()
            for t in range(LT):
                yt = y[:, 128 * t:128 * (t + 1)] * gt_
                out_v[pl.ds(base, 16), pl.ds(128 * t, 128)] = (h[t] + ys[t] + jnp.where(is_sel, yt, 0.0)).astype(bf16)
            fix = pltpu.make_async_copy(out_v.at[pl.ds(base, 16), :], out_hbm.at[pl.ds(base, 16), :], sems.at[2 * NB + 7])
            fix.start()
            fix.wait()
        else:
            out_copy(out_lo, NB).start()
            started.append((out_lo, NB))
            for (lo, hi) in started:
                out_copy(lo, hi).wait()

    @jax.jit
    def fn(A_x, A_wqkv, A_wo, B_x, B_w_r, B_w_gate, B_w_up, B_w_down):
        x = A_x.reshape(S, D)
        wr = B_w_r.astype(f32).reshape(1, D)
        anyspec = pl.BlockSpec(memory_space=pl.ANY)
        out = pl.pallas_call(
            kern,
            out_shape=jax.ShapeDtypeStruct((S, D), bf16),
            in_specs=[pl.BlockSpec(memory_space=pltpu.SMEM), anyspec, anyspec, anyspec, pl.BlockSpec(memory_space=pltpu.VMEM), anyspec, anyspec, anyspec],
            out_specs=anyspec,
            scratch_shapes=[
                pltpu.VMEM((S, D), bf16),
                pltpu.VMEM((3, D, D), bf16),
                pltpu.VMEM((D, D), bf16),
                pltpu.VMEM((D, F), bf16), pltpu.VMEM((D, F), bf16), pltpu.VMEM((F, D), bf16),
                pltpu.VMEM((S, D), bf16),
                pltpu.VMEM((D // 2, 3 * D), i32),
                pltpu.VMEM((D // 2, D), i32),
                pltpu.VMEM((LT, D, 128), f32),
                pltpu.VMEM((S // 2, D), i32),
                pltpu.VMEM((S // 2, D), i32),
                pltpu.VMEM((LT, S, 128), f32),
                pltpu.VMEM((LT, S, 128), f32),
                pltpu.VMEM((LT, S + HALO, 128), f32),
                pltpu.VMEM((LT, S + HALO, 128), f32),
                pltpu.VMEM((LT, S, 128), f32),
                pltpu.SemaphoreType.DMA((2 * NB + 8,)),
            ],
            compiler_params=pltpu.CompilerParams(vmem_limit_bytes=100 * 2**20, flags=({k: True for k in flags.split("+")} if flags else None)),
            name="fused",
        )(np.zeros((1,), np.int32), x, A_wqkv, A_wo, wr, B_w_gate, B_w_up, B_w_down)
        return out.reshape(1, S, D)

    return fn


pallas_sequential_preLN__sliding_local_dilated__moe_arch_mod__prompt_kernel = make_kernel()
```

```python
import functools
import numpy as np
import jax
import jax.numpy as jnp
from jax import lax
import jax.experimental.pallas as pl
import jax.experimental.pallas.tpu as pltpu

S, D, H, DH, F = 2048, 640, 32, 20, 1536
NW, DIL = 8, 2
LT = D // 128
HALO = 16
f32, bf16, i32 = jnp.float32, jnp.bfloat16, jnp.int32
LOG2E = 1.4426950408889634


def make_kernel(T=256, flags=None, RA=8, dk=1, df=7, bars="058", simple=False, order="wq", ffn=True, pb=1, stag=0):
    NB = S // T

    def kern(z_ref, x_hbm, wqkv_hbm, wo_hbm, wr_ref, wg_hbm, wu_hbm, wd_hbm, out_hbm,
             x_v, wq_v, wo_v, wg_v, wu_v, wd_v, out_v,
             wp, wop, wof, xn, os_, xf, hall, qs, ks, vs, sems, *blk):
        P = functools.partial
        z = z_ref[0]
        qkb = blk[:NB]
        vb = blk[NB:2 * NB]
        xnb = blk[2 * NB:3 * NB]
        osb = blk[3 * NB:4 * NB]
        xfb = blk[4 * NB:5 * NB]

        def x_copy(i):
            return pltpu.make_async_copy(x_hbm.at[pl.ds(i * T, T), :], x_v.at[pl.ds(i * T, T), :], sems.at[i])
        def out_copy(lo, hi):
            return pltpu.make_async_copy(out_v.at[pl.ds(lo * T, (hi - lo) * T), :], out_hbm.at[pl.ds(lo * T, (hi - lo) * T), :], sems.at[NB + lo])
        w_copies = [pltpu.make_async_copy(wqkv_hbm.at[:, pl.ds(s * D, D)], wq_v.at[s], sems.at[2 * NB + s]) for s in range(3)]
        wo_copy = pltpu.make_async_copy(wo_hbm, wo_v, sems.at[2 * NB + 3])
        wg_copy = pltpu.make_async_copy(wg_hbm, wg_v, sems.at[2 * NB + 4])
        wu_copy = pltpu.make_async_copy(wu_hbm, wu_v, sems.at[2 * NB + 5])
        wd_copy = pltpu.make_async_copy(wd_hbm, wd_v, sems.at[2 * NB + 6])
        x_copy(0).start()
        w_copies[0].start()
        if stag == 0:
            w_copies[1].start()
            x_copy(1).start()
            w_copies[2].start()
            wo_copy.start()
            for i in range(2, NB):
                x_copy(i).start()
            if ffn:
                wg_copy.start(); wu_copy.start(); wd_copy.start()

        def dma_stage(k):
            if stag == 0:
                return
            if k == 0:
                w_copies[1].start()
            elif k == 1:
                w_copies[2].start()
                x_copy(1).start()
            elif k == 2:
                wo_copy.start()
                for i in range(2, NB):
                    x_copy(i).start()
                if stag == 1 and ffn:
                    wg_copy.start(); wu_copy.start(); wd_copy.start()
            elif k == 3:
                if stag == 2 and ffn:
                    wg_copy.start(); wu_copy.start(); wd_copy.start()

        lane = lax.broadcasted_iota(i32, (8, 128), 1)
        never = (lane + z) < 0
        alltok, marks, done = [], [], [0]

        def permute_w(sec):
            hh = lane & 31
            gg = lane >> 5
            for t in range(LT):
                c = hh * DH + 4 * t + gg
                src_lane = c & 127
                hp = (13 * ((lane >> 2) - t)) & 31
                cp = hp * DH + 4 * t + (lane & 3)
                tile_l = cp >> 7
                for r in range(D // 16):
                    srcs = [pltpu.bitcast(wq_v[sec, pl.ds(16 * r, 16), pl.ds(128 * u, 128)], i32) for u in range(LT)]
                    comb = srcs[0]
                    for u in range(1, LT):
                        comb = jnp.where(tile_l == u, srcs[u], comb)
                    wp[pl.ds(8 * r, 8), pl.ds(128 * (sec * LT + t), 128)] = jnp.take_along_axis(comb, src_lane, axis=1)

        def permute_wo():
            for u in range(LT):
                wof[u] = wo_v[:, pl.ds(128 * u, 128)].astype(f32)
            for u in range(LT):
                for d in range(DH):
                    blk_ = wof[u, pl.ds(d, H, stride=DH), :]
                    wop[pl.ds(16 * d, 16), pl.ds(128 * u, 128)] = pltpu.bitcast(blk_.astype(bf16), i32)

        def red(f, xs):
            a = xs[0]
            for b in xs[1:]:
                a = f(a, b)
            return a

        def ln(xs):
            s = xs[0]
            for a in xs[1:]:
                s = s + a
            m = jnp.sum(s, axis=1, keepdims=True) * (1.0 / D)
            cs = [a - m for a in xs]
            q = cs[0] * cs[0]
            for a in cs[1:]:
                q = q + a * a
            var = jnp.sum(q, axis=1, keepdims=True) * (1.0 / D)
            rs = lax.rsqrt(var + 1e-5)
            return [a * rs for a in cs]

        def s1_chunk(r0):
            xs = [x_v[pl.ds(r0, 16), pl.ds(128 * t, 128)].astype(f32) for t in range(LT)]
            ys = ln(xs)
            for t in range(LT):
                i, rr_ = divmod(r0, T)
                if pb & 4:
                    xnb[i][pl.ds(rr_ // 2, 8), pl.ds(128 * t, 128)] = pltpu.bitcast(ys[t].astype(bf16), i32)
                else:
                    xn[pl.ds(r0 // 2, 8), pl.ds(128 * t, 128)] = pltpu.bitcast(ys[t].astype(bf16), i32)
                if pb & 16:
                    xfb[i][t, pl.ds(rr_, 16), :] = xs[t]
                else:
                    xf[t, pl.ds(r0, 16), :] = xs[t]
            if df & 2:
                alltok.append(ys[LT - 1][8:16])

        def lhs(buf, i):
            if buf is xn and pb & 4:
                a = xnb[i][...]
            elif buf is os_ and pb & 8:
                a = osb[i][...]
            else:
                a = buf[pl.ds(i * T // 2, T // 2), :]
            marks.append(len(alltok))
            if len(marks) > dk:
                lo, hi = done[0], marks[-dk - 1]
                if hi > lo:
                    tk = alltok[lo]
                    for t_ in alltok[lo + 1:hi]:
                        tk = jnp.maximum(tk, t_)
                    a00 = jnp.where(never, lax.bitcast_convert_type(tk, i32), a[0:8, 0:128])
                    a = jnp.concatenate([jnp.concatenate([a00, a[0:8, 128:]], axis=1), a[8:]], axis=0)
                done[0] = hi
            return pltpu.bitcast(a, bf16)

        def s2_unit(i, n):
            sec, t = divmod(n, LT)
            res = jnp.dot(lhs(xn, i), pltpu.bitcast(wp[:, pl.ds(128 * n, 128)], bf16), preferred_element_type=f32)
            if sec == 0:
                res = res * (DH ** -0.5 * LOG2E)
            if sec < 2 and pb & 1:
                qkb[i][sec, t, pl.ds(HALO, T), :] = res
                if sec > 0 and i + 1 < NB:
                    qkb[i + 1][sec, t, pl.ds(0, HALO), :] = res[T - HALO:, :]
            elif sec == 2 and pb & 2:
                vb[i][t, pl.ds(HALO, T), :] = res
                if i + 1 < NB:
                    vb[i + 1][t, pl.ds(0, HALO), :] = res[T - HALO:, :]
            elif sec == 0:
                qs[t, pl.ds(i * T, T), :] = res
            elif sec == 1:
                ks[t, pl.ds(HALO + i * T, T), :] = res
            else:
                vs[t, pl.ds(HALO + i * T, T), :] = res

        o8 = {}

        def s3_rows(r0, R):
            masked = r0 < HALO
            i, rr_ = divmod(r0, T)
            if pb & 1:
                q = [qkb[i][0, t, pl.ds(HALO + rr_, R), :] for t in range(LT)]
                kl = lambda t, w: qkb[i][1, t, pl.ds(HALO + rr_ - DIL * w, R), :]
            else:
                q = [qs[t, pl.ds(r0, R), :] for t in range(LT)]
                kl = lambda t, w: ks[t, pl.ds(HALO + r0 - DIL * w, R), :]
            if pb & 2:
                vl = lambda t, w: vb[i][t, pl.ds(HALO + rr_ - DIL * w, R), :]
            else:
                vl = lambda t, w: vs[t, pl.ds(HALO + r0 - DIL * w, R), :]
            Ls = []
            for w in range(NW):
                p = red(jnp.add, [q[t] * kl(t, w) for t in range(LT)])
                p = p + pltpu.roll(p, 64, 1)
                p = p + pltpu.roll(p, 32, 1)
                if masked and w > 0:
                    row = lax.broadcasted_iota(i32, (R, 128), 0) + r0
                    p = jnp.where(row >= DIL * w, p, -1e9)
                Ls.append(p)
            m = red(jnp.maximum, Ls)
            es = [jnp.exp2(l - m) for l in Ls]
            inv = 1.0 / red(jnp.add, es)
            for t in range(LT):
                a = red(jnp.add, [es[w] * vl(t, w) for w in range(NW)]) * inv
                if R >= 16:
                    os_[pl.ds(r0 // 2, R // 2), pl.ds(128 * t, 128)] = pltpu.bitcast(a.astype(bf16), i32)
                else:
                    o8[t] = o8.get(t, []) + [a]
                    if len(o8[t]) == 2:
                        ov = pltpu.bitcast(jnp.concatenate(o8[t], axis=0).astype(bf16), i32)
                        if pb & 8:
                            osb[i][pl.ds((rr_ - 8) // 2, 8), pl.ds(128 * t, 128)] = ov
                        else:
                            os_[pl.ds((r0 - 8) // 2, 8), pl.ds(128 * t, 128)] = ov
                        o8[t] = []
            if df & 1:
                alltok.append(a[0:8])

        wr2 = wr_ref[...].astype(f32).reshape(1, D)
        wr = [wr2[:, 128 * t:128 * (t + 1)] for t in range(LT)]
        best = [None, None]

        def s4_unit(i, n):
            res = jnp.dot(lhs(os_, i), pltpu.bitcast(wop[:, pl.ds(128 * n, 128)], bf16), preferred_element_type=f32)
            hall[n, pl.ds(i * T, T), :] = res + (xfb[i][n] if pb & 16 else xf[n, pl.ds(i * T, T), :])

        def s4_chunk(r0):
            h = [hall[t, pl.ds(r0, 16), :] for t in range(LT)]
            ys = ln(h)
            rr = ys[0] * wr[0]
            for t in range(1, LT):
                rr = rr + ys[t] * wr[t]
            rv = jnp.broadcast_to(jnp.sum(rr, axis=1, keepdims=True), (16, 128))
            idx = lax.broadcasted_iota(i32, (16, 128), 0) + r0
            if best[0] is None:
                best[0], best[1] = rv, idx
            else:
                gt = rv > best[0]
                best[0] = jnp.where(gt, rv, best[0])
                best[1] = jnp.where(gt, idx, best[1])
            for t in range(LT):
                o_ = h[t] + ys[t]
                out_v[pl.ds(r0, 16), pl.ds(128 * t, 128)] = o_.astype(bf16)
            if df & 4:
                alltok.append(o_[8:16])

        def merge(pools):
            tot = sum(len(p) for p in pools)
            idx = [0] * len(pools)
            mix = []
            for s in range(tot):
                bp, bv = None, None
                for pi, p in enumerate(pools):
                    if idx[pi] < len(p):
                        v = (idx[pi] + 0.5) / len(p)
                        if bv is None or v < bv:
                            bp, bv = pi, v
                mix.append(pools[bp][idx[bp]])
                idx[bp] += 1
            return mix

        def interleave(units, chunks):
            nu, nc = len(units), len(chunks)
            done_ = 0
            for u, fu in enumerate(units):
                fu()
                tgt = (u + 1) * nc // nu
                while done_ < tgt:
                    chunks[done_]()
                    done_ += 1
            while done_ < nc:
                chunks[done_]()
                done_ += 1

        for t in range(LT):
            ks[t, pl.ds(0, HALO), :] = jnp.zeros((HALO, 128), f32)
            vs[t, pl.ds(0, HALO), :] = jnp.zeros((HALO, 128), f32)
            qkb[0][1, t, pl.ds(0, HALO), :] = jnp.zeros((HALO, 128), f32)
            vb[0][t, pl.ds(0, HALO), :] = jnp.zeros((HALO, 128), f32)

        barl = [int(c) for c in bars]
        x_done = [0]
        def wait_x(upto):
            while x_done[0] < min(upto, NB):
                x_copy(x_done[0]).wait()
                x_done[0] += 1
        if simple:
            wait_x(NB)
            for c in w_copies:
                c.wait()
            wo_copy.wait()
            for sec in range(3):
                permute_w(sec)
            permute_wo()
        else:
            wait_x(1)
            dma_stage(0)
        for r in range(T // 16):
            s1_chunk(16 * r)
        started = []
        out_lo = 0
        for j in range(-1, NB + 2):
            if j in barl and not simple:
                nxt = [b for b in barl if b > j]
                wait_x((nxt[0] if nxt else NB) + 2)
                if j == barl[0]:
                    wo_copy.wait()
                    dma_stage(3)
            if j in barl and j - 2 > out_lo:
                out_copy(out_lo, j - 2).start()
                started.append((out_lo, j - 2))
                out_lo = j - 2
            wo_units = [P(s4_unit, j - 1, n) for n in range(LT)] if 0 <= j - 1 < NB else []
            qkv_units = []
            if 0 <= j + 1 < NB:
                if j == -1 and not simple:
                    for sec in range(3):
                        qkv_units.append(w_copies[sec].wait)
                        if sec < 2:
                            qkv_units.append(P(dma_stage, sec + 1))
                        if sec == 2:
                            qkv_units.append(P(wait_x, 2))
                        qkv_units.append(P(permute_w, sec))
                        qkv_units += [P(s2_unit, 0, sec * LT + t) for t in range(LT)]
                else:
                    qkv_units = [P(s2_unit, j + 1, n) for n in range(3 * LT)]
            att = [P(s3_rows, j * T + RA * r, RA) for r in range(T // RA)] if 0 <= j < NB else []
            ln1 = [P(s1_chunk, (j + 2) * T + 16 * r) for r in range(T // 16)] if 0 <= j + 2 < NB else []
            ln2 = [P(s4_chunk, (j - 2) * T + 16 * r) for r in range(T // 16)] if 0 <= j - 2 < NB else []
            extra = [permute_wo] if (j == 0 and not simple) else []
            chunks = merge([att, ln2, ln1, extra])
            if j == -1 and not simple:
                for fu in qkv_units:
                    fu()
                for c in chunks:
                    c()
                continue
            if order == "wq":
                units = wo_units + qkv_units
            elif order == "qw":
                units = qkv_units + wo_units
            else:
                units = qkv_units[:10] + wo_units + qkv_units[10:]
            if units:
                interleave(units, chunks)
            else:
                for c in chunks:
                    c()

        if ffn:
            mx = jnp.max(best[0])
            sel = jnp.min(jnp.where(best[0] == mx, best[1], S))
            base = pl.multiple_of((sel >> 4) << 4, 16)
            h = [hall[t, pl.ds(base, 16), :] for t in range(LT)]
            ys = ln(h)
            row = lax.broadcasted_iota(i32, (16, 128), 0) + base
            is_sel = row == sel
            xs = jnp.concatenate([jnp.where(is_sel, y, 0.0) for y in ys], axis=1)
            xs = jnp.broadcast_to(jnp.sum(xs, axis=0, keepdims=True), (16, D)).astype(bf16)
            wg_copy.wait(); wu_copy.wait(); wd_copy.wait()
            out_copy(out_lo, NB).start()
            started.append((out_lo, NB))
            g = jnp.dot(xs, wg_v[...], preferred_element_type=f32)
            u = jnp.dot(xs, wu_v[...], preferred_element_type=f32)
            a = (g * jax.nn.sigmoid(g) * u).astype(bf16)
            y = jnp.dot(a, wd_v[...], preferred_element_type=f32)
            gt_ = jax.nn.sigmoid(jnp.full((16, 128), mx, f32))
            for (lo, hi) in started:
                out_copy(lo, hi).wait()
            for t in range(LT):
                yt = y[:, 128 * t:128 * (t + 1)] * gt_
                out_v[pl.ds(base, 16), pl.ds(128 * t, 128)] = (h[t] + (ys[t] + jnp.where(is_sel, yt, 0.0))).astype(bf16)
            fix = pltpu.make_async_copy(out_v.at[pl.ds(base, 16), :], out_hbm.at[pl.ds(base, 16), :], sems.at[2 * NB + 7])
            fix.start()
            fix.wait()
        else:
            out_copy(out_lo, NB).start()
            started.append((out_lo, NB))
            for (lo, hi) in started:
                out_copy(lo, hi).wait()

    @jax.jit
    def fn(A_x, A_wqkv, A_wo, B_x, B_w_r, B_w_gate, B_w_up, B_w_down):
        x = A_x.reshape(S, D)
        anyspec = pl.BlockSpec(memory_space=pl.ANY)
        out = pl.pallas_call(
            kern,
            out_shape=jax.ShapeDtypeStruct((S, D), bf16),
            in_specs=[pl.BlockSpec(memory_space=pltpu.SMEM), anyspec, anyspec, anyspec, pl.BlockSpec(memory_space=pltpu.VMEM), anyspec, anyspec, anyspec],
            out_specs=anyspec,
            scratch_shapes=[
                pltpu.VMEM((S, D), bf16),
                pltpu.VMEM((3, D, D), bf16),
                pltpu.VMEM((D, D), bf16),
                pltpu.VMEM((D, F), bf16), pltpu.VMEM((D, F), bf16), pltpu.VMEM((F, D), bf16),
                pltpu.VMEM((S, D), bf16),
                pltpu.VMEM((D // 2, 3 * D), i32),
                pltpu.VMEM((D // 2, D), i32),
                pltpu.VMEM((LT, D, 128), f32),
                pltpu.VMEM((S // 2, D), i32),
                pltpu.VMEM((S // 2, D), i32),
                pltpu.VMEM((LT, S, 128), f32),
                pltpu.VMEM((LT, S, 128), f32),
                pltpu.VMEM((LT, S, 128), f32),
                pltpu.VMEM((LT, S + HALO, 128), f32),
                pltpu.VMEM((LT, S + HALO, 128), f32),
                pltpu.SemaphoreType.DMA((2 * NB + 8,)),
            ] + [pltpu.VMEM((2, LT, T + HALO + 8, 128), f32) for _ in range(NB)]
              + [pltpu.VMEM((LT, T + HALO + 8, 128), f32) for _ in range(NB)]
              + [pltpu.VMEM((T // 2, D), i32) for _ in range(2 * NB)]
              + [pltpu.VMEM((LT, T, 128), f32) for _ in range(NB)],
            compiler_params=pltpu.CompilerParams(vmem_limit_bytes=100 * 2**20, flags=({k: True for k in flags.split("+")} if flags else None)),
            name="fused",
        )(np.zeros((1,), np.int32), x, A_wqkv, A_wo, B_w_r, B_w_gate, B_w_up, B_w_down)
        return out.reshape(1, S, D)

    return fn


pallas_sequential_preLN__sliding_local_dilated__moe_arch_mod__prompt_kernel = make_kernel()
```

```python
import functools
import numpy as np
import jax
import jax.numpy as jnp
from jax import lax
import jax.experimental.pallas as pl
import jax.experimental.pallas.tpu as pltpu

S, D, H, DH, F = 2048, 640, 32, 20, 1536
NW, DIL = 8, 2
LT = D // 128
HALO = 16
f32, bf16, i32 = jnp.float32, jnp.bfloat16, jnp.int32
LOG2E = 1.4426950408889634


def make_kernel(T=256, flags=None, RA=8, dk=1, df=7, bars="01579", simple=False, order="wq", ffn=True, pb=1, stag=0, pro=2, pq=2):
    NB = S // T

    def kern(z_ref, x_hbm, wqkv_hbm, wo_hbm, wr_ref, wg_hbm, wu_hbm, wd_hbm, out_hbm,
             x_v, wq_v, wo_v, wg_v, wu_v, wd_v, out_v,
             wp, wop, wof, xn, os_, xf, hall, qs, ks, vs, sems, *blk):
        P = functools.partial
        z = z_ref[0]
        qkb = blk[:NB]
        vb = blk[NB:2 * NB]
        xnb = blk[2 * NB:3 * NB]
        osb = blk[3 * NB:4 * NB]
        xfb = blk[4 * NB:5 * NB]

        def x_copy(i):
            return pltpu.make_async_copy(x_hbm.at[pl.ds(i * T, T), :], x_v.at[pl.ds(i * T, T), :], sems.at[i])
        def out_copy(lo, hi):
            return pltpu.make_async_copy(out_v.at[pl.ds(lo * T, (hi - lo) * T), :], out_hbm.at[pl.ds(lo * T, (hi - lo) * T), :], sems.at[NB + lo])
        w_copies = [pltpu.make_async_copy(wqkv_hbm.at[:, pl.ds(s * D, D)], wq_v.at[s], sems.at[2 * NB + s]) for s in range(3)]
        wo_copy = pltpu.make_async_copy(wo_hbm, wo_v, sems.at[2 * NB + 3])
        wg_copy = pltpu.make_async_copy(wg_hbm, wg_v, sems.at[2 * NB + 4])
        wu_copy = pltpu.make_async_copy(wu_hbm, wu_v, sems.at[2 * NB + 5])
        wd_copy = pltpu.make_async_copy(wd_hbm, wd_v, sems.at[2 * NB + 6])
        x_copy(0).start()
        w_copies[0].start()
        if stag == 0:
            w_copies[1].start()
            x_copy(1).start()
            w_copies[2].start()
            x_copy(2).start()
            wo_copy.start()
            for i in range(3, NB):
                x_copy(i).start()
            if ffn:
                wg_copy.start(); wu_copy.start(); wd_copy.start()

        def dma_stage(k):
            if stag == 0:
                return
            if k == 0:
                w_copies[1].start()
            elif k == 1:
                w_copies[2].start()
                x_copy(1).start()
            elif k == 2:
                wo_copy.start()
                for i in range(2, NB):
                    x_copy(i).start()
                if stag == 1 and ffn:
                    wg_copy.start(); wu_copy.start(); wd_copy.start()
            elif k == 3:
                if stag == 2 and ffn:
                    wg_copy.start(); wu_copy.start(); wd_copy.start()

        lane = lax.broadcasted_iota(i32, (8, 128), 1)
        never = (lane + z) < 0
        alltok, marks, done = [], [], [0]

        def permute_w(sec):
            hh = lane & 31
            gg = lane >> 5
            for t in range(LT):
                c = hh * DH + 4 * t + gg
                src_lane = c & 127
                hp = (13 * ((lane >> 2) - t)) & 31
                cp = hp * DH + 4 * t + (lane & 3)
                tile_l = cp >> 7
                for r in range(D // 16):
                    srcs = [pltpu.bitcast(wq_v[sec, pl.ds(16 * r, 16), pl.ds(128 * u, 128)], i32) for u in range(LT)]
                    comb = srcs[0]
                    for u in range(1, LT):
                        comb = jnp.where(tile_l == u, srcs[u], comb)
                    wp[pl.ds(8 * r, 8), pl.ds(128 * (sec * LT + t), 128)] = jnp.take_along_axis(comb, src_lane, axis=1)

        def permute_chunks(sec, nch=3):
            hh = lane & 31
            gg = lane >> 5
            consts = []
            for t in range(LT):
                c = hh * DH + 4 * t + gg
                hp = (13 * ((lane >> 2) - t)) & 31
                cp = hp * DH + 4 * t + (lane & 3)
                consts.append((c & 127, cp >> 7))
            def chunk(r_lo, r_hi):
                for r in range(r_lo, r_hi):
                    srcs = [pltpu.bitcast(wq_v[sec, pl.ds(16 * r, 16), pl.ds(128 * u, 128)], i32) for u in range(LT)]
                    for t in range(LT):
                        src_lane, tile_l = consts[t]
                        comb = srcs[0]
                        for u in range(1, LT):
                            comb = jnp.where(tile_l == u, srcs[u], comb)
                        g = jnp.take_along_axis(comb, src_lane, axis=1)
                        wp[pl.ds(8 * r, 8), pl.ds(128 * (sec * LT + t), 128)] = g
                alltok.append(lax.bitcast_convert_type(g, f32))
            n = D // 16
            return [P(chunk, k * n // nch, (k + 1) * n // nch) for k in range(nch)]

        def permute_tile(sec, t):
            c = (lane & 31) * DH + 4 * t + (lane >> 5)
            hp = (13 * ((lane >> 2) - t)) & 31
            tile_l = (hp * DH + 4 * t + (lane & 3)) >> 7
            src_lane = c & 127
            for r in range(D // 16):
                srcs = [pltpu.bitcast(wq_v[sec, pl.ds(16 * r, 16), pl.ds(128 * u, 128)], i32) for u in range(LT)]
                comb = srcs[0]
                for u in range(1, LT):
                    comb = jnp.where(tile_l == u, srcs[u], comb)
                wp[pl.ds(8 * r, 8), pl.ds(128 * (sec * LT + t), 128)] = jnp.take_along_axis(comb, src_lane, axis=1)

        def permute_wo():
            for u in range(LT):
                wof[u] = wo_v[:, pl.ds(128 * u, 128)].astype(f32)
            for u in range(LT):
                for d in range(DH):
                    blk_ = wof[u, pl.ds(d, H, stride=DH), :]
                    wop[pl.ds(16 * d, 16), pl.ds(128 * u, 128)] = pltpu.bitcast(blk_.astype(bf16), i32)

        def red(f, xs):
            a = xs[0]
            for b in xs[1:]:
                a = f(a, b)
            return a

        def ln(xs):
            s = xs[0]
            for a in xs[1:]:
                s = s + a
            m = jnp.sum(s, axis=1, keepdims=True) * (1.0 / D)
            cs = [a - m for a in xs]
            q = cs[0] * cs[0]
            for a in cs[1:]:
                q = q + a * a
            var = jnp.sum(q, axis=1, keepdims=True) * (1.0 / D)
            rs = lax.rsqrt(var + 1e-5)
            return [a * rs for a in cs]

        def s1_chunk(r0):
            xs = [x_v[pl.ds(r0, 16), pl.ds(128 * t, 128)].astype(f32) for t in range(LT)]
            ys = ln(xs)
            for t in range(LT):
                i, rr_ = divmod(r0, T)
                if pb & 4:
                    xnb[i][pl.ds(rr_ // 2, 8), pl.ds(128 * t, 128)] = pltpu.bitcast(ys[t].astype(bf16), i32)
                else:
                    xn[pl.ds(r0 // 2, 8), pl.ds(128 * t, 128)] = pltpu.bitcast(ys[t].astype(bf16), i32)
                if pb & 16:
                    xfb[i][t, pl.ds(rr_, 16), :] = xs[t]
                else:
                    xf[t, pl.ds(r0, 16), :] = xs[t]
            if df & 2:
                alltok.append(ys[LT - 1][8:16])

        def lhs(buf, i):
            if buf is xn and pb & 4:
                a = xnb[i][...]
            elif buf is os_ and pb & 8:
                a = osb[i][...]
            else:
                a = buf[pl.ds(i * T // 2, T // 2), :]
            marks.append(len(alltok))
            if len(marks) > dk:
                lo, hi = done[0], marks[-dk - 1]
                if hi > lo:
                    tk = alltok[lo]
                    for t_ in alltok[lo + 1:hi]:
                        tk = jnp.maximum(tk, t_)
                    a00 = jnp.where(never, lax.bitcast_convert_type(tk, i32), a[0:8, 0:128])
                    a = jnp.concatenate([jnp.concatenate([a00, a[0:8, 128:]], axis=1), a[8:]], axis=0)
                done[0] = hi
            return pltpu.bitcast(a, bf16)

        def s2_unit(i, n):
            sec, t = divmod(n, LT)
            res = jnp.dot(lhs(xn, i), pltpu.bitcast(wp[:, pl.ds(128 * n, 128)], bf16), preferred_element_type=f32)
            if sec == 0:
                res = res * (DH ** -0.5 * LOG2E)
            if sec < 2 and pb & 1:
                qkb[i][sec, t, pl.ds(HALO, T), :] = res
                if sec > 0 and i + 1 < NB:
                    qkb[i + 1][sec, t, pl.ds(0, HALO), :] = res[T - HALO:, :]
            elif sec == 2 and pb & 2:
                vb[i][t, pl.ds(HALO, T), :] = res
                if i + 1 < NB:
                    vb[i + 1][t, pl.ds(0, HALO), :] = res[T - HALO:, :]
            elif sec == 0:
                qs[t, pl.ds(i * T, T), :] = res
            elif sec == 1:
                ks[t, pl.ds(HALO + i * T, T), :] = res
            else:
                vs[t, pl.ds(HALO + i * T, T), :] = res

        o8 = {}

        def s3_rows(r0, R):
            masked = r0 < HALO
            i, rr_ = divmod(r0, T)
            if pb & 1:
                q = [qkb[i][0, t, pl.ds(HALO + rr_, R), :] for t in range(LT)]
                kl = lambda t, w: qkb[i][1, t, pl.ds(HALO + rr_ - DIL * w, R), :]
            else:
                q = [qs[t, pl.ds(r0, R), :] for t in range(LT)]
                kl = lambda t, w: ks[t, pl.ds(HALO + r0 - DIL * w, R), :]
            if pb & 2:
                vl = lambda t, w: vb[i][t, pl.ds(HALO + rr_ - DIL * w, R), :]
            else:
                vl = lambda t, w: vs[t, pl.ds(HALO + r0 - DIL * w, R), :]
            Ls = []
            for w in range(NW):
                p = red(jnp.add, [q[t] * kl(t, w) for t in range(LT)])
                p = p + pltpu.roll(p, 64, 1)
                p = p + pltpu.roll(p, 32, 1)
                if masked and w > 0:
                    row = lax.broadcasted_iota(i32, (R, 128), 0) + r0
                    p = jnp.where(row >= DIL * w, p, -1e9)
                Ls.append(p)
            m = red(jnp.maximum, Ls)
            es = [jnp.exp2(l - m) for l in Ls]
            inv = 1.0 / red(jnp.add, es)
            for t in range(LT):
                a = red(jnp.add, [es[w] * vl(t, w) for w in range(NW)]) * inv
                if R >= 16:
                    os_[pl.ds(r0 // 2, R // 2), pl.ds(128 * t, 128)] = pltpu.bitcast(a.astype(bf16), i32)
                else:
                    o8[t] = o8.get(t, []) + [a]
                    if len(o8[t]) == 2:
                        ov = pltpu.bitcast(jnp.concatenate(o8[t], axis=0).astype(bf16), i32)
                        if pb & 8:
                            osb[i][pl.ds((rr_ - 8) // 2, 8), pl.ds(128 * t, 128)] = ov
                        else:
                            os_[pl.ds((r0 - 8) // 2, 8), pl.ds(128 * t, 128)] = ov
                        o8[t] = []
            if df & 1:
                alltok.append(a[0:8])

        wr2 = wr_ref[...].astype(f32).reshape(1, D)
        wr = [wr2[:, 128 * t:128 * (t + 1)] for t in range(LT)]
        best = [None, None]

        def s4_unit(i, n):
            res = jnp.dot(lhs(os_, i), pltpu.bitcast(wop[:, pl.ds(128 * n, 128)], bf16), preferred_element_type=f32)
            hall[n, pl.ds(i * T, T), :] = res + (xfb[i][n] if pb & 16 else xf[n, pl.ds(i * T, T), :])

        def s4_chunk(r0):
            h = [hall[t, pl.ds(r0, 16), :] for t in range(LT)]
            ys = ln(h)
            rr = ys[0] * wr[0]
            for t in range(1, LT):
                rr = rr + ys[t] * wr[t]
            rv = jnp.broadcast_to(jnp.sum(rr, axis=1, keepdims=True), (16, 128))
            idx = lax.broadcasted_iota(i32, (16, 128), 0) + r0
            if best[0] is None:
                best[0], best[1] = rv, idx
            else:
                gt = rv > best[0]
                best[0] = jnp.where(gt, rv, best[0])
                best[1] = jnp.where(gt, idx, best[1])
            for t in range(LT):
                o_ = h[t] + ys[t]
                out_v[pl.ds(r0, 16), pl.ds(128 * t, 128)] = o_.astype(bf16)
            if df & 4:
                alltok.append(o_[8:16])

        def merge(pools):
            tot = sum(len(p) for p in pools)
            idx = [0] * len(pools)
            mix = []
            for s in range(tot):
                bp, bv = None, None
                for pi, p in enumerate(pools):
                    if idx[pi] < len(p):
                        v = (idx[pi] + 0.5) / len(p)
                        if bv is None or v < bv:
                            bp, bv = pi, v
                mix.append(pools[bp][idx[bp]])
                idx[bp] += 1
            return mix

        def interleave(units, chunks):
            nu, nc = len(units), len(chunks)
            done_ = 0
            for u, fu in enumerate(units):
                fu()
                tgt = (u + 1) * nc // nu
                while done_ < tgt:
                    chunks[done_]()
                    done_ += 1
            while done_ < nc:
                chunks[done_]()
                done_ += 1

        for t in range(LT):
            ks[t, pl.ds(0, HALO), :] = jnp.zeros((HALO, 128), f32)
            vs[t, pl.ds(0, HALO), :] = jnp.zeros((HALO, 128), f32)
            qkb[0][1, t, pl.ds(0, HALO), :] = jnp.zeros((HALO, 128), f32)
            vb[0][t, pl.ds(0, HALO), :] = jnp.zeros((HALO, 128), f32)

        barl = [int(c) for c in bars]
        x_done = [0]
        def wait_x(upto):
            while x_done[0] < min(upto, NB):
                x_copy(x_done[0]).wait()
                x_done[0] += 1
        if simple:
            wait_x(NB)
            for c in w_copies:
                c.wait()
            wo_copy.wait()
            for sec in range(3):
                permute_w(sec)
            permute_wo()
        else:
            wait_x(1)
            dma_stage(0)
        for r in range(T // 16):
            s1_chunk(16 * r)
        started = []
        out_lo = 0
        for j in range(-1, NB + 2):
            if j in barl and not simple:
                nxt = [b for b in barl if b > j]
                wait_x((nxt[0] if nxt else NB) + 2)
                if j == barl[0]:
                    wo_copy.wait()
                    dma_stage(3)
            if j in barl and j - 2 > out_lo:
                out_copy(out_lo, j - 2).start()
                started.append((out_lo, j - 2))
                out_lo = j - 2
            wo_units = [P(s4_unit, j - 1, n) for n in range(LT)] if 0 <= j - 1 < NB else []
            qkv_units = []
            if 0 <= j + 1 < NB:
                if j == -1 and not simple:
                    for sec in range(3):
                        qkv_units.append(w_copies[sec].wait)
                        if sec < 2:
                            qkv_units.append(P(dma_stage, sec + 1))
                        if sec == 2:
                            qkv_units.append(P(wait_x, 2))
                        qkv_units.append(P(permute_w, sec))
                        qkv_units += [P(s2_unit, 0, sec * LT + t) for t in range(LT)]
                else:
                    qkv_units = [P(s2_unit, j + 1, n) for n in range(3 * LT)]
            att = [P(s3_rows, j * T + RA * r, RA) for r in range(T // RA)] if 0 <= j < NB else []
            ln1 = [P(s1_chunk, (j + 2) * T + 16 * r) for r in range(T // 16)] if 0 <= j + 2 < NB else []
            ln2 = [P(s4_chunk, (j - 2) * T + 16 * r) for r in range(T // 16)] if 0 <= j - 2 < NB else []
            extra = [permute_wo] if (j == 0 and not simple) else []
            chunks = merge([att, ln2, ln1, extra])
            if j == -1 and not simple and pro == 2:
                for sec in range(3):
                    w_copies[sec].wait(); dma_stage(sec + 1)
                    if sec == 2:
                        wait_x(2)
                    us = []
                    for t in range(LT):
                        us += [lambda sec=sec, t=t: (permute_tile(sec, t), s2_unit(0, sec * LT + t))]
                    if sec < 2:
                        for fu in us:
                            fu()
                    else:
                        interleave(us, chunks)
                continue
            if j == -1 and not simple and pro:
                U = [P(s2_unit, 0, n) for n in range(3 * LT)]
                w_copies[0].wait(); dma_stage(1)
                for c in permute_chunks(0, 1):
                    c()
                for fu in U[0:pq]:
                    fu()
                w_copies[1].wait(); dma_stage(2)
                interleave(U[pq:5], permute_chunks(1, 5 - pq))
                for fu in U[5:5 + pq]:
                    fu()
                w_copies[2].wait(); wait_x(2)
                interleave(U[5 + pq:10], permute_chunks(2, 5 - pq))
                interleave(U[10:15], chunks)
                continue
            if j == -1 and not simple:
                for fu in qkv_units:
                    fu()
                for c in chunks:
                    c()
                continue
            if order == "wq":
                units = wo_units + qkv_units
            elif order == "qw":
                units = qkv_units + wo_units
            else:
                units = qkv_units[:10] + wo_units + qkv_units[10:]
            if units:
                interleave(units, chunks)
            else:
                for c in chunks:
                    c()

        if ffn:
            mx = jnp.max(best[0])
            sel = jnp.min(jnp.where(best[0] == mx, best[1], S))
            base = pl.multiple_of((sel >> 4) << 4, 16)
            h = [hall[t, pl.ds(base, 16), :] for t in range(LT)]
            ys = ln(h)
            row = lax.broadcasted_iota(i32, (16, 128), 0) + base
            is_sel = row == sel
            xs = jnp.concatenate([jnp.where(is_sel, y, 0.0) for y in ys], axis=1)
            xs = jnp.broadcast_to(jnp.sum(xs, axis=0, keepdims=True), (16, D)).astype(bf16)
            wg_copy.wait(); wu_copy.wait(); wd_copy.wait()
            out_copy(out_lo, NB).start()
            started.append((out_lo, NB))
            g = jnp.dot(xs, wg_v[...], preferred_element_type=f32)
            u = jnp.dot(xs, wu_v[...], preferred_element_type=f32)
            a = (g * jax.nn.sigmoid(g) * u).astype(bf16)
            y = jnp.dot(a, wd_v[...], preferred_element_type=f32)
            gt_ = jax.nn.sigmoid(jnp.full((16, 128), mx, f32))
            for (lo, hi) in started:
                out_copy(lo, hi).wait()
            for t in range(LT):
                yt = y[:, 128 * t:128 * (t + 1)] * gt_
                out_v[pl.ds(base, 16), pl.ds(128 * t, 128)] = (h[t] + (ys[t] + jnp.where(is_sel, yt, 0.0))).astype(bf16)
            fix = pltpu.make_async_copy(out_v.at[pl.ds(base, 16), :], out_hbm.at[pl.ds(base, 16), :], sems.at[2 * NB + 7])
            fix.start()
            fix.wait()
        else:
            out_copy(out_lo, NB).start()
            started.append((out_lo, NB))
            for (lo, hi) in started:
                out_copy(lo, hi).wait()

    @jax.jit
    def fn(A_x, A_wqkv, A_wo, B_x, B_w_r, B_w_gate, B_w_up, B_w_down):
        x = A_x.reshape(S, D)
        anyspec = pl.BlockSpec(memory_space=pl.ANY)
        out = pl.pallas_call(
            kern,
            out_shape=jax.ShapeDtypeStruct((S, D), bf16),
            in_specs=[pl.BlockSpec(memory_space=pltpu.SMEM), anyspec, anyspec, anyspec, pl.BlockSpec(memory_space=pltpu.VMEM), anyspec, anyspec, anyspec],
            out_specs=anyspec,
            scratch_shapes=[
                pltpu.VMEM((S, D), bf16),
                pltpu.VMEM((3, D, D), bf16),
                pltpu.VMEM((D, D), bf16),
                pltpu.VMEM((D, F), bf16), pltpu.VMEM((D, F), bf16), pltpu.VMEM((F, D), bf16),
                pltpu.VMEM((S, D), bf16),
                pltpu.VMEM((D // 2, 3 * D), i32),
                pltpu.VMEM((D // 2, D), i32),
                pltpu.VMEM((LT, D, 128), f32),
                pltpu.VMEM((S // 2, D), i32),
                pltpu.VMEM((S // 2, D), i32),
                pltpu.VMEM((LT, S, 128), f32),
                pltpu.VMEM((LT, S, 128), f32),
                pltpu.VMEM((LT, S, 128), f32),
                pltpu.VMEM((LT, S + HALO, 128), f32),
                pltpu.VMEM((LT, S + HALO, 128), f32),
                pltpu.SemaphoreType.DMA((2 * NB + 8,)),
            ] + [pltpu.VMEM((2, LT, T + HALO + 8, 128), f32) for _ in range(NB)]
              + [pltpu.VMEM((LT, T + HALO + 8, 128), f32) for _ in range(NB)]
              + [pltpu.VMEM((T // 2, D), i32) for _ in range(2 * NB)]
              + [pltpu.VMEM((LT, T, 128), f32) for _ in range(NB)],
            compiler_params=pltpu.CompilerParams(vmem_limit_bytes=100 * 2**20, flags=({k: True for k in flags.split("+")} if flags else None)),
            name="fused",
        )(np.zeros((1,), np.int32), x, A_wqkv, A_wo, B_w_r, B_w_gate, B_w_up, B_w_down)
        return out.reshape(1, S, D)

    return fn


pallas_sequential_preLN__sliding_local_dilated__moe_arch_mod__prompt_kernel = make_kernel()
```

```python
import functools
import numpy as np
import jax
import jax.numpy as jnp
from jax import lax
import jax.experimental.pallas as pl
import jax.experimental.pallas.tpu as pltpu

S, D, H, DH, F = 2048, 640, 32, 20, 1536
NW, DIL = 8, 2
LT = D // 128
HALO = 16
f32, bf16, i32 = jnp.float32, jnp.bfloat16, jnp.int32
LOG2E = 1.4426950408889634


def make_kernel(T=256, flags=None, RA=8, dk=1, df=7, bars="01579", simple=False, order="mid", ffn=True, pb=1, stag=0, pro=2, pq=2, spec=1, split=2):
    NB = S // T

    def kern(z_ref, x_hbm, wqkv_hbm, wo_hbm, wr_ref, wg_hbm, wu_hbm, wd_hbm, out_hbm,
             x_v, wq_v, wo_v, wg_v, wu_v, wd_v, out_v,
             wp, wop, wof, xn, os_, xf, hall, qs, ks, vs, fixbuf, base_s, sems, *blk):
        P = functools.partial
        z = z_ref[0]
        qkb = blk[:NB]
        vb = blk[NB:2 * NB]
        xnb = blk[2 * NB:3 * NB]
        osb = blk[3 * NB:4 * NB]
        xfb = blk[4 * NB:5 * NB]

        def x_copy(i):
            return pltpu.make_async_copy(x_hbm.at[pl.ds(i * T, T), :], x_v.at[pl.ds(i * T, T), :], sems.at[i])
        def out_copy(lo, hi):
            return pltpu.make_async_copy(out_v.at[pl.ds(lo * T, (hi - lo) * T), :], out_hbm.at[pl.ds(lo * T, (hi - lo) * T), :], sems.at[NB + lo])
        w_copies = [pltpu.make_async_copy(wqkv_hbm.at[:, pl.ds(s * D, D)], wq_v.at[s], sems.at[2 * NB + s]) for s in range(3)]
        wo_copy = pltpu.make_async_copy(wo_hbm, wo_v, sems.at[2 * NB + 3])
        wg_copy = pltpu.make_async_copy(wg_hbm, wg_v, sems.at[2 * NB + 4])
        wu_copy = pltpu.make_async_copy(wu_hbm, wu_v, sems.at[2 * NB + 5])
        wd_copy = pltpu.make_async_copy(wd_hbm, wd_v, sems.at[2 * NB + 6])
        x_copy(0).start()
        w_copies[0].start()
        if stag == 0:
            w_copies[1].start()
            x_copy(1).start()
            w_copies[2].start()
            x_copy(2).start()
            wo_copy.start()
            for i in range(3, NB):
                x_copy(i).start()
            if ffn:
                wg_copy.start(); wu_copy.start(); wd_copy.start()

        def dma_stage(k):
            if stag == 0:
                return
            if k == 0:
                w_copies[1].start()
            elif k == 1:
                w_copies[2].start()
                x_copy(1).start()
            elif k == 2:
                wo_copy.start()
                for i in range(2, NB):
                    x_copy(i).start()
                if stag == 1 and ffn:
                    wg_copy.start(); wu_copy.start(); wd_copy.start()
            elif k == 3:
                if stag == 2 and ffn:
                    wg_copy.start(); wu_copy.start(); wd_copy.start()

        lane = lax.broadcasted_iota(i32, (8, 128), 1)
        never = (lane + z) < 0
        alltok, marks, done = [], [], [0]

        def permute_w(sec):
            hh = lane & 31
            gg = lane >> 5
            for t in range(LT):
                c = hh * DH + 4 * t + gg
                src_lane = c & 127
                hp = (13 * ((lane >> 2) - t)) & 31
                cp = hp * DH + 4 * t + (lane & 3)
                tile_l = cp >> 7
                for r in range(D // 16):
                    srcs = [pltpu.bitcast(wq_v[sec, pl.ds(16 * r, 16), pl.ds(128 * u, 128)], i32) for u in range(LT)]
                    comb = srcs[0]
                    for u in range(1, LT):
                        comb = jnp.where(tile_l == u, srcs[u], comb)
                    wp[pl.ds(8 * r, 8), pl.ds(128 * (sec * LT + t), 128)] = jnp.take_along_axis(comb, src_lane, axis=1)

        def permute_chunks(sec, nch=3):
            hh = lane & 31
            gg = lane >> 5
            consts = []
            for t in range(LT):
                c = hh * DH + 4 * t + gg
                hp = (13 * ((lane >> 2) - t)) & 31
                cp = hp * DH + 4 * t + (lane & 3)
                consts.append((c & 127, cp >> 7))
            def chunk(r_lo, r_hi):
                for r in range(r_lo, r_hi):
                    srcs = [pltpu.bitcast(wq_v[sec, pl.ds(16 * r, 16), pl.ds(128 * u, 128)], i32) for u in range(LT)]
                    for t in range(LT):
                        src_lane, tile_l = consts[t]
                        comb = srcs[0]
                        for u in range(1, LT):
                            comb = jnp.where(tile_l == u, srcs[u], comb)
                        g = jnp.take_along_axis(comb, src_lane, axis=1)
                        wp[pl.ds(8 * r, 8), pl.ds(128 * (sec * LT + t), 128)] = g
                alltok.append(lax.bitcast_convert_type(g, f32))
            n = D // 16
            return [P(chunk, k * n // nch, (k + 1) * n // nch) for k in range(nch)]

        def permute_tile(sec, t):
            c = (lane & 31) * DH + 4 * t + (lane >> 5)
            hp = (13 * ((lane >> 2) - t)) & 31
            tile_l = (hp * DH + 4 * t + (lane & 3)) >> 7
            src_lane = c & 127
            for r in range(D // 16):
                srcs = [pltpu.bitcast(wq_v[sec, pl.ds(16 * r, 16), pl.ds(128 * u, 128)], i32) for u in range(LT)]
                comb = srcs[0]
                for u in range(1, LT):
                    comb = jnp.where(tile_l == u, srcs[u], comb)
                wp[pl.ds(8 * r, 8), pl.ds(128 * (sec * LT + t), 128)] = jnp.take_along_axis(comb, src_lane, axis=1)

        def permute_wo():
            for u in range(LT):
                wof[u] = wo_v[:, pl.ds(128 * u, 128)].astype(f32)
            for u in range(LT):
                for d in range(DH):
                    blk_ = wof[u, pl.ds(d, H, stride=DH), :]
                    wop[pl.ds(16 * d, 16), pl.ds(128 * u, 128)] = pltpu.bitcast(blk_.astype(bf16), i32)

        def red(f, xs):
            a = xs[0]
            for b in xs[1:]:
                a = f(a, b)
            return a

        def ln(xs):
            s = xs[0]
            for a in xs[1:]:
                s = s + a
            m = jnp.sum(s, axis=1, keepdims=True) * (1.0 / D)
            cs = [a - m for a in xs]
            q = cs[0] * cs[0]
            for a in cs[1:]:
                q = q + a * a
            var = jnp.sum(q, axis=1, keepdims=True) * (1.0 / D)
            rs = lax.rsqrt(var + 1e-5)
            return [a * rs for a in cs]

        def s1_chunk(r0):
            xs = [x_v[pl.ds(r0, 16), pl.ds(128 * t, 128)].astype(f32) for t in range(LT)]
            ys = ln(xs)
            for t in range(LT):
                i, rr_ = divmod(r0, T)
                if pb & 4:
                    xnb[i][pl.ds(rr_ // 2, 8), pl.ds(128 * t, 128)] = pltpu.bitcast(ys[t].astype(bf16), i32)
                else:
                    xn[pl.ds(r0 // 2, 8), pl.ds(128 * t, 128)] = pltpu.bitcast(ys[t].astype(bf16), i32)
                if pb & 16:
                    xfb[i][t, pl.ds(rr_, 16), :] = xs[t]
                else:
                    xf[t, pl.ds(r0, 16), :] = xs[t]
            if df & 2:
                alltok.append(ys[LT - 1][8:16])

        def lhs(buf, i):
            if buf is xn and pb & 4:
                a = xnb[i][...]
            elif buf is os_ and pb & 8:
                a = osb[i][...]
            else:
                a = buf[pl.ds(i * T // 2, T // 2), :]
            marks.append(len(alltok))
            if len(marks) > dk:
                lo, hi = done[0], marks[-dk - 1]
                if hi > lo:
                    tk = alltok[lo]
                    for t_ in alltok[lo + 1:hi]:
                        tk = jnp.maximum(tk, t_)
                    a00 = jnp.where(never, lax.bitcast_convert_type(tk, i32), a[0:8, 0:128])
                    a = jnp.concatenate([jnp.concatenate([a00, a[0:8, 128:]], axis=1), a[8:]], axis=0)
                done[0] = hi
            return pltpu.bitcast(a, bf16)

        def s2_unit(i, n):
            sec, t = divmod(n, LT)
            res = jnp.dot(lhs(xn, i), pltpu.bitcast(wp[:, pl.ds(128 * n, 128)], bf16), preferred_element_type=f32)
            if sec == 0:
                res = res * (DH ** -0.5 * LOG2E)
            if sec < 2 and pb & 1:
                qkb[i][sec, t, pl.ds(HALO, T), :] = res
                if sec > 0 and i + 1 < NB:
                    qkb[i + 1][sec, t, pl.ds(0, HALO), :] = res[T - HALO:, :]
            elif sec == 2 and pb & 2:
                vb[i][t, pl.ds(HALO, T), :] = res
                if i + 1 < NB:
                    vb[i + 1][t, pl.ds(0, HALO), :] = res[T - HALO:, :]
            elif sec == 0:
                qs[t, pl.ds(i * T, T), :] = res
            elif sec == 1:
                ks[t, pl.ds(HALO + i * T, T), :] = res
            else:
                vs[t, pl.ds(HALO + i * T, T), :] = res

        o8 = {}

        def s3_rows(r0, R):
            masked = r0 < HALO
            i, rr_ = divmod(r0, T)
            if pb & 1:
                q = [qkb[i][0, t, pl.ds(HALO + rr_, R), :] for t in range(LT)]
                kl = lambda t, w: qkb[i][1, t, pl.ds(HALO + rr_ - DIL * w, R), :]
            else:
                q = [qs[t, pl.ds(r0, R), :] for t in range(LT)]
                kl = lambda t, w: ks[t, pl.ds(HALO + r0 - DIL * w, R), :]
            if pb & 2:
                vl = lambda t, w: vb[i][t, pl.ds(HALO + rr_ - DIL * w, R), :]
            else:
                vl = lambda t, w: vs[t, pl.ds(HALO + r0 - DIL * w, R), :]
            Ls = []
            for w in range(NW):
                p = red(jnp.add, [q[t] * kl(t, w) for t in range(LT)])
                p = p + pltpu.roll(p, 64, 1)
                p = p + pltpu.roll(p, 32, 1)
                if masked and w > 0:
                    row = lax.broadcasted_iota(i32, (R, 128), 0) + r0
                    p = jnp.where(row >= DIL * w, p, -1e9)
                Ls.append(p)
            m = red(jnp.maximum, Ls)
            es = [jnp.exp2(l - m) for l in Ls]
            inv = 1.0 / red(jnp.add, es)
            for t in range(LT):
                a = red(jnp.add, [es[w] * vl(t, w) for w in range(NW)]) * inv
                if R >= 16:
                    os_[pl.ds(r0 // 2, R // 2), pl.ds(128 * t, 128)] = pltpu.bitcast(a.astype(bf16), i32)
                else:
                    o8[t] = o8.get(t, []) + [a]
                    if len(o8[t]) == 2:
                        ov = pltpu.bitcast(jnp.concatenate(o8[t], axis=0).astype(bf16), i32)
                        if pb & 8:
                            osb[i][pl.ds((rr_ - 8) // 2, 8), pl.ds(128 * t, 128)] = ov
                        else:
                            os_[pl.ds((r0 - 8) // 2, 8), pl.ds(128 * t, 128)] = ov
                        o8[t] = []
            if df & 1:
                alltok.append(a[0:8])

        wr2 = wr_ref[...].astype(f32).reshape(1, D)
        wr = [wr2[:, 128 * t:128 * (t + 1)] for t in range(LT)]
        best = [None, None]

        def s4_unit(i, n):
            res = jnp.dot(lhs(os_, i), pltpu.bitcast(wop[:, pl.ds(128 * n, 128)], bf16), preferred_element_type=f32)
            hall[n, pl.ds(i * T, T), :] = res + (xfb[i][n] if pb & 16 else xf[n, pl.ds(i * T, T), :])

        def s4_sub(r0, R):
            res = jnp.dot(pltpu.bitcast(os_[pl.ds(r0 // 2, R // 2), :], bf16), pltpu.bitcast(wop[...], bf16), preferred_element_type=f32)
            for n in range(LT):
                hall[n, pl.ds(r0, R), :] = res[:, 128 * n:128 * (n + 1)] + xf[n, pl.ds(r0, R), :]

        def s4_chunk(r0):
            h = [hall[t, pl.ds(r0, 16), :] for t in range(LT)]
            ys = ln(h)
            rr = ys[0] * wr[0]
            for t in range(1, LT):
                rr = rr + ys[t] * wr[t]
            rv = jnp.broadcast_to(jnp.sum(rr, axis=1, keepdims=True), (16, 128))
            idx = lax.broadcasted_iota(i32, (16, 128), 0) + r0
            if best[0] is None:
                best[0], best[1] = rv, idx
            else:
                gt = rv > best[0]
                best[0] = jnp.where(gt, rv, best[0])
                best[1] = jnp.where(gt, idx, best[1])
            for t in range(LT):
                o_ = h[t] + ys[t]
                out_v[pl.ds(r0, 16), pl.ds(128 * t, 128)] = o_.astype(bf16)
            if df & 4:
                alltok.append(o_[8:16])

        def wait_ffn():
            wg_copy.wait(); wu_copy.wait(); wd_copy.wait()

        def ffn_fix(mx, sel):
            base = pl.multiple_of((sel >> 4) << 4, 16)
            h = [hall[t, pl.ds(base, 16), :] for t in range(LT)]
            ys = ln(h)
            row = lax.broadcasted_iota(i32, (16, 128), 0) + base
            is_sel = row == sel
            xs = jnp.concatenate([jnp.where(is_sel, y, 0.0) for y in ys], axis=1)
            xs = jnp.broadcast_to(jnp.sum(xs, axis=0, keepdims=True), (16, D)).astype(bf16)
            g = jnp.dot(xs, wg_v[...], preferred_element_type=f32)
            u = jnp.dot(xs, wu_v[...], preferred_element_type=f32)
            a = (g * jax.nn.sigmoid(g) * u).astype(bf16)
            y = jnp.dot(a, wd_v[...], preferred_element_type=f32)
            gt_ = jax.nn.sigmoid(jnp.full((16, 128), mx, f32))
            for t in range(LT):
                yt = y[:, 128 * t:128 * (t + 1)] * gt_
                fixbuf[:, pl.ds(128 * t, 128)] = (h[t] + (ys[t] + jnp.where(is_sel, yt, 0.0))).astype(bf16)
            base_s[0] = base

        spec_mx = [None]

        def merge(pools):
            tot = sum(len(p) for p in pools)
            idx = [0] * len(pools)
            mix = []
            for s in range(tot):
                bp, bv = None, None
                for pi, p in enumerate(pools):
                    if idx[pi] < len(p):
                        v = (idx[pi] + 0.5) / len(p)
                        if bv is None or v < bv:
                            bp, bv = pi, v
                mix.append(pools[bp][idx[bp]])
                idx[bp] += 1
            return mix

        def interleave(units, chunks):
            nu, nc = len(units), len(chunks)
            done_ = 0
            for u, fu in enumerate(units):
                fu()
                tgt = (u + 1) * nc // nu
                while done_ < tgt:
                    chunks[done_]()
                    done_ += 1
            while done_ < nc:
                chunks[done_]()
                done_ += 1

        for t in range(LT):
            ks[t, pl.ds(0, HALO), :] = jnp.zeros((HALO, 128), f32)
            vs[t, pl.ds(0, HALO), :] = jnp.zeros((HALO, 128), f32)
            qkb[0][1, t, pl.ds(0, HALO), :] = jnp.zeros((HALO, 128), f32)
            vb[0][t, pl.ds(0, HALO), :] = jnp.zeros((HALO, 128), f32)

        barl = [int(c) for c in bars]
        x_done = [0]
        def wait_x(upto):
            while x_done[0] < min(upto, NB):
                x_copy(x_done[0]).wait()
                x_done[0] += 1
        if simple:
            wait_x(NB)
            for c in w_copies:
                c.wait()
            wo_copy.wait()
            for sec in range(3):
                permute_w(sec)
            permute_wo()
        else:
            wait_x(1)
            dma_stage(0)
        for r in range(T // 16):
            s1_chunk(16 * r)
        started = []
        out_lo = 0
        for j in range(-1, NB + 2):
            if j in barl and not simple:
                nxt = [b for b in barl if b > j]
                wait_x((nxt[0] if nxt else NB) + 2)
                if j == barl[0]:
                    wo_copy.wait()
                    dma_stage(3)
            if j in barl and j - 2 > out_lo:
                out_copy(out_lo, j - 2).start()
                started.append((out_lo, j - 2))
                out_lo = j - 2
            if spec and ffn and j == NB + 1:
                wait_ffn()
                smx = jnp.max(best[0])
                spec_mx[0] = smx
                ffn_fix(smx, jnp.min(jnp.where(best[0] == smx, best[1], S)))
            wo_units = [P(s4_unit, j - 1, n) for n in range(LT)] if 0 <= j - 1 < NB else []
            qkv_units = []
            if 0 <= j + 1 < NB:
                if j == -1 and not simple:
                    for sec in range(3):
                        qkv_units.append(w_copies[sec].wait)
                        if sec < 2:
                            qkv_units.append(P(dma_stage, sec + 1))
                        if sec == 2:
                            qkv_units.append(P(wait_x, 2))
                        qkv_units.append(P(permute_w, sec))
                        qkv_units += [P(s2_unit, 0, sec * LT + t) for t in range(LT)]
                else:
                    qkv_units = [P(s2_unit, j + 1, n) for n in range(3 * LT)]
            att = [P(s3_rows, j * T + RA * r, RA) for r in range(T // RA)] if 0 <= j < NB else []
            ln1 = [P(s1_chunk, (j + 2) * T + 16 * r) for r in range(T // 16)] if 0 <= j + 2 < NB else []
            ln2 = [P(s4_chunk, (j - 2) * T + 16 * r) for r in range(T // 16)] if 0 <= j - 2 < NB else []
            extra = [permute_wo] if (j == 0 and not simple) else []
            chunks = merge([att, ln2, ln1, extra])
            if split and j == NB:
                R = T // split
                for c in chunks:
                    c()
                for g in range(split):
                    s4_sub((NB - 1) * T + g * R, R)
                    if g < split - 1:
                        for r in range(R // 16):
                            s4_chunk((NB - 1) * T + g * R + 16 * r)
                continue
            if split and j == NB + 1:
                R = T // split
                for r in range(R // 16):
                    s4_chunk((NB - 1) * T + (split - 1) * R + 16 * r)
                continue
            if j == -1 and not simple and pro == 3:
                us = [lambda n=n: (permute_tile(n // LT, n % LT), s2_unit(0, n)) for n in range(3 * LT)]
                w_copies[0].wait(); dma_stage(1)
                for fu in us[0:pq]:
                    fu()
                w_copies[1].wait(); dma_stage(2)
                for fu in us[pq:LT + pq]:
                    fu()
                w_copies[2].wait(); wait_x(2); dma_stage(3)
                rest_u = us[LT + pq:]
                interleave(rest_u, chunks)
                continue
            if j == -1 and not simple and pro == 2:
                for sec in range(3):
                    w_copies[sec].wait(); dma_stage(sec + 1)
                    if sec == 2:
                        wait_x(2)
                    us = []
                    for t in range(LT):
                        us += [lambda sec=sec, t=t: (permute_tile(sec, t), s2_unit(0, sec * LT + t))]
                    if sec < 2:
                        for fu in us:
                            fu()
                    else:
                        interleave(us, chunks)
                continue
            if j == -1 and not simple and pro:
                U = [P(s2_unit, 0, n) for n in range(3 * LT)]
                w_copies[0].wait(); dma_stage(1)
                for c in permute_chunks(0, 1):
                    c()
                for fu in U[0:pq]:
                    fu()
                w_copies[1].wait(); dma_stage(2)
                interleave(U[pq:5], permute_chunks(1, 5 - pq))
                for fu in U[5:5 + pq]:
                    fu()
                w_copies[2].wait(); wait_x(2)
                interleave(U[5 + pq:10], permute_chunks(2, 5 - pq))
                interleave(U[10:15], chunks)
                continue
            if j == -1 and not simple:
                for fu in qkv_units:
                    fu()
                for c in chunks:
                    c()
                continue
            if order == "wq":
                units = wo_units + qkv_units
            elif order == "qw":
                units = qkv_units + wo_units
            else:
                units = qkv_units[:10] + wo_units + qkv_units[10:]
            if units:
                interleave(units, chunks)
            else:
                for c in chunks:
                    c()

        if ffn:
            out_copy(out_lo, NB).start()
            started.append((out_lo, NB))
            mx = jnp.max(best[0])
            if spec:
                @pl.when(mx > spec_mx[0])
                def _():
                    ffn_fix(mx, jnp.min(jnp.where(best[0] == mx, best[1], S)))
            else:
                wait_ffn()
                ffn_fix(mx, jnp.min(jnp.where(best[0] == mx, best[1], S)))
            for (lo, hi) in started:
                out_copy(lo, hi).wait()
            base = pl.multiple_of(base_s[0], 16)
            fix = pltpu.make_async_copy(fixbuf, out_hbm.at[pl.ds(base, 16), :], sems.at[2 * NB + 7])
            fix.start()
            fix.wait()
        else:
            out_copy(out_lo, NB).start()
            started.append((out_lo, NB))
            for (lo, hi) in started:
                out_copy(lo, hi).wait()

    @jax.jit
    def fn(A_x, A_wqkv, A_wo, B_x, B_w_r, B_w_gate, B_w_up, B_w_down):
        x = A_x.reshape(S, D)
        anyspec = pl.BlockSpec(memory_space=pl.ANY)
        out = pl.pallas_call(
            kern,
            out_shape=jax.ShapeDtypeStruct((S, D), bf16),
            in_specs=[pl.BlockSpec(memory_space=pltpu.SMEM), anyspec, anyspec, anyspec, pl.BlockSpec(memory_space=pltpu.VMEM), anyspec, anyspec, anyspec],
            out_specs=anyspec,
            scratch_shapes=[
                pltpu.VMEM((S, D), bf16),
                pltpu.VMEM((3, D, D), bf16),
                pltpu.VMEM((D, D), bf16),
                pltpu.VMEM((D, F), bf16), pltpu.VMEM((D, F), bf16), pltpu.VMEM((F, D), bf16),
                pltpu.VMEM((S, D), bf16),
                pltpu.VMEM((D // 2, 3 * D), i32),
                pltpu.VMEM((D // 2, D), i32),
                pltpu.VMEM((LT, D, 128), f32),
                pltpu.VMEM((S // 2, D), i32),
                pltpu.VMEM((S // 2, D), i32),
                pltpu.VMEM((LT, S, 128), f32),
                pltpu.VMEM((LT, S, 128), f32),
                pltpu.VMEM((LT, S, 128), f32),
                pltpu.VMEM((LT, S + HALO, 128), f32),
                pltpu.VMEM((LT, S + HALO, 128), f32),
                pltpu.VMEM((16, D), bf16),
                pltpu.SMEM((1,), i32),
                pltpu.SemaphoreType.DMA((2 * NB + 8,)),
            ] + [pltpu.VMEM((2, LT, T + HALO + 8, 128), f32) for _ in range(NB)]
              + [pltpu.VMEM((LT, T + HALO + 8, 128), f32) for _ in range(NB)]
              + [pltpu.VMEM((T // 2, D), i32) for _ in range(2 * NB)]
              + [pltpu.VMEM((LT, T, 128), f32) for _ in range(NB)],
            compiler_params=pltpu.CompilerParams(vmem_limit_bytes=100 * 2**20, flags=({k: True for k in flags.split("+")} if flags else None)),
            name="fused",
        )(np.zeros((1,), np.int32), x, A_wqkv, A_wo, B_w_r, B_w_gate, B_w_up, B_w_down)
        return out.reshape(1, S, D)

    return fn


pallas_sequential_preLN__sliding_local_dilated__moe_arch_mod__prompt_kernel = make_kernel()
```
